```python
import jax
import jax.numpy as jnp

def _softmax(x, axis=-1):
    return jax.nn.softmax(x, axis=axis)
def _gelu(x):
    return jax.nn.gelu(x, approximate=True)
def _silu(x):
    return jax.nn.silu(x)
def _sigmoid(x):
    return jax.nn.sigmoid(x)
def _layernorm(x, axis=-1, eps=1e-5):
    m = jnp.mean(x, axis=axis, keepdims=True)
    v = jnp.var(x, axis=axis, keepdims=True)
    return (x - m) / jnp.sqrt(v + eps)
def _scatter_add(tgt, idx, src, axis=0):
    return tgt.at[idx].add(src)
def _segment_sum(src, seg, n):
    return jax.ops.segment_sum(src, seg, n)
class _Rng:
    def __init__(self, key):
        self._k = key
    def _next(self):
        self._k, sub = jax.random.split(self._k)
        return sub
    def normal(self, shape):
        return jax.random.normal(self._next(), shape, dtype=jnp.bfloat16)
    def randint(self, lo, hi, shape):
        return jax.random.randint(self._next(), shape, lo, hi, dtype=jnp.int32)
    def uniform(self, shape, lo=0.0, hi=1.0):
        return jax.random.uniform(self._next(), shape, jnp.bfloat16, lo, hi)
    def permutation(self, n):
        return jax.random.permutation(self._next(), n)


kernel_name = 'recurrent_scan__compressed_kv_cla__dense_activation_gelu__decode'

def setup_inputs():
    _rng = _Rng(jax.random.key(int.from_bytes(__import__("os").urandom(4), "little")))
    _w = (lambda a: (lambda t: t.astype(jnp.bfloat16) if jnp.issubdtype(t.dtype, jnp.floating) else t)(jnp.asarray(a)))
    def _A_setup():
        B, H, Sq, Sk, D, M = 2, 32, 1, 16384, 128, 512
        Dc = 4 * D
        return {
            "x": _w((lambda *s: _rng.normal(s) * 0.05)(B, Sq, M)),
            "c_kv": _w((lambda *s: _rng.normal(s) * 0.05)(B, Sk, Dc)),
            "w_q": _w((lambda *s: _rng.normal(s) * 0.05)(M, H, D) * (M ** -0.5)),
            "w_uk": _w((lambda *s: _rng.normal(s) * 0.05)(Dc, H, D) * (Dc ** -0.5)),
            "w_uv": _w((lambda *s: _rng.normal(s) * 0.05)(Dc, H, D) * (Dc ** -0.5)),
            "w_o": _w((lambda *s: _rng.normal(s) * 0.05)(H, D, M) * ((H * D) ** -0.5)),
        }
    _A_in = _A_setup()

    def _B_setup():
        B, S, D, F = 2, 1, 512, 1792
        return {
            "x": _w((lambda *s: _rng.normal(s) * 0.05)(B, S, D)),
            "w1": _w((lambda *s: _rng.normal(s) * 0.05)(D, F) * (D ** -0.5)),
            "b1": _w((lambda *s: _rng.normal(s) * 0.05)(F) * 0.01),
            "w2": _w((lambda *s: _rng.normal(s) * 0.05)(F, D) * (F ** -0.5)),
            "b2": _w((lambda *s: _rng.normal(s) * 0.05)(D) * 0.01),
        }
    _B_in = _B_setup()

    return {
        "A_x": _A_in["x"],
        "A_c_kv": _A_in["c_kv"],
        "A_w_q": _A_in["w_q"],
        "A_w_uk": _A_in["w_uk"],
        "A_w_uv": _A_in["w_uv"],
        "A_w_o": _A_in["w_o"],
        "B_x": _B_in["x"],
        "B_w1": _B_in["w1"],
        "B_b1": _B_in["b1"],
        "B_w2": _B_in["w2"],
        "B_b2": _B_in["b2"],
    }

def reference(A_x, A_c_kv, A_w_q, A_w_uk, A_w_uv, A_w_o, B_x, B_w1, B_b1, B_w2, B_b2):
    def _A_ref(x, c_kv, w_q, w_uk, w_uv, w_o):
        B, Sq, M = x.shape[0], x.shape[1], x.shape[2]
        Sk = c_kv.shape[1]
        H, D = w_q.shape[1], w_q.shape[2]
        q = jnp.einsum("bqm,mhd->bhqd", x, w_q)
        k = jnp.einsum("bkc,chd->bhkd", c_kv, w_uk)
        v = jnp.einsum("bkc,chd->bhkd", c_kv, w_uv)
        scores = jnp.einsum("bhqd,bhkd->bhqk", q, k) * (D ** -0.5)
        off = Sk - Sq
        qi = jnp.arange(Sq)[:, None]
        kj = jnp.arange(Sk)[None, :]
        cmask = kj <= (qi + off)
        scores = jnp.where(cmask[None, None], scores, -1e9)
        p = _softmax(scores, axis=-1)
        ctx = jnp.einsum("bhqk,bhkd->bhqd", p, v)
        return jnp.einsum("bhqd,hdm->bqm", ctx, w_o)

    def _B_ref(x, w1, b1, w2, b2):
        h = jnp.einsum("bsd,df->bsf", x, w1) + b1
        h = _gelu(h)
        return jnp.einsum("bsf,fd->bsd", h, w2) + b2

    x = A_x
    xn = _layernorm(x, axis=-1)
    s = _A_ref(xn, A_c_kv, A_w_q, A_w_uk, A_w_uv, A_w_o)
    g = _silu(_B_ref(xn, B_w1, B_b1, B_w2, B_b2))
    return x + s * g
```

```python
import contextlib
import jax
import jax.numpy as jnp
from jax import lax
import jax.experimental.pallas as pl
import jax.experimental.pallas.tpu as pltpu

B, H, D, M, SK, DC, F = 2, 32, 128, 512, 16384, 512, 1792
F32, BF16 = jnp.float32, jnp.bfloat16


def make_kernel(CH=2048, TB=512, WO_CHUNKS=8, scopes=False):
    NCH = SK // CH
    NB = CH // TB
    HPC = H // WO_CHUNKS

    def scope(name):
        return jax.named_scope(name) if scopes else contextlib.nullcontext()

    def kernel(x_hbm, ckv_hbm, wq_hbm, wuk_hbm, wuv_hbm, wo_hbm, w1_hbm, b1_hbm, w2_hbm, b2_hbm,
               o_ref,
               x_v, b1_v, b2_v, wq_v, wuk_v, ckv_v, wuv_v, w1_v, w2_v, wo_v,
               sems):
        cp_x = pltpu.make_async_copy(x_hbm, x_v, sems.at[0])
        cp_b1 = pltpu.make_async_copy(b1_hbm, b1_v, sems.at[1])
        cp_b2 = pltpu.make_async_copy(b2_hbm, b2_v, sems.at[2])
        cp_wq = pltpu.make_async_copy(wq_hbm, wq_v, sems.at[3])
        cp_wuk = pltpu.make_async_copy(wuk_hbm, wuk_v, sems.at[4])
        cp_wuv = pltpu.make_async_copy(wuv_hbm, wuv_v, sems.at[5])
        cp_w1 = pltpu.make_async_copy(w1_hbm, w1_v, sems.at[6])
        cp_w2 = pltpu.make_async_copy(w2_hbm, w2_v, sems.at[7])

        def cp_c(i):
            return pltpu.make_async_copy(ckv_hbm.at[pl.ds(i * CH, CH)], ckv_v.at[pl.ds(i * CH, CH)], sems.at[8 + i])

        def cp_o(i):
            n = HPC * D
            return pltpu.make_async_copy(wo_hbm.at[pl.ds(i * n, n)], wo_v.at[pl.ds(i * n, n)], sems.at[8 + B * NCH + i])

        cp_x.start()
        cp_wq.start()
        cp_b1.start()
        cp_b2.start()
        cp_wuk.start()
        for i in range(B * NCH):
            cp_c(i).start()
        cp_wuv.start()
        cp_w1.start()
        cp_w2.start()
        for i in range(WO_CHUNKS):
            cp_o(i).start()

        r_i = lax.broadcasted_iota(jnp.int32, (128, 256), 0)
        c_i = lax.broadcasted_iota(jnp.int32, (128, 256), 1)
        E0 = jnp.where((c_i >> 1) == r_i, 1.0, 0.0).astype(BF16)
        r_j = lax.broadcasted_iota(jnp.int32, (256, 128), 0)
        c_j = lax.broadcasted_iota(jnp.int32, (256, 128), 1)
        F0 = jnp.where((r_j >> 1) == c_j, 1.0, 0.0).astype(BF16)
        row16 = lax.broadcasted_iota(jnp.int32, (16, 1024), 0)
        lane16 = lax.broadcasted_iota(jnp.int32, (16, 1024), 1)
        par_mask = (row16 & 1) == (lane16 & 1)

        def expand2(a_bf16):
            return jnp.concatenate(
                [jnp.dot(a_bf16[:, 128 * t:128 * (t + 1)], E0, preferred_element_type=F32) for t in range(4)], axis=1)

        with scope("ln"):
            cp_x.wait()
            x = x_v[...].astype(F32)
            mu = jnp.mean(x, axis=-1, keepdims=True)
            xc = x - mu
            var = jnp.mean(xc * xc, axis=-1, keepdims=True)
            xn = xc / jnp.sqrt(var + 1e-5)
            xn16 = jnp.concatenate([jnp.broadcast_to(xn[0:1], (8, M)), jnp.broadcast_to(xn[1:2], (8, M))], axis=0)
            xn16_bf = xn16.astype(BF16)
            x16 = jnp.where(par_mask, expand2(xn16_bf), 0.0).astype(BF16)

        row128 = lax.broadcasted_iota(jnp.int32, (16, 128), 0) & 7
        with scope("wait_wq"):
            cp_wq.wait()
        with scope("q"):
            wq32 = wq_v.bitcast(jnp.uint32)
            qs = []
            for g in range(4):
                acc = None
                for ii in range(4):
                    i = 4 * g + ii
                    w = pltpu.bitcast(wq32[pl.ds(i, M, stride=16), :], BF16)
                    o = jnp.dot(x16, w, preferred_element_type=F32)
                    o = jnp.where((row128 >> 1) == ii, o, 0.0)
                    acc = o if acc is None else acc + o
                qs.append(acc.astype(BF16))

        with scope("wait_wuk"):
            cp_wuk.wait()
        with scope("qabs"):
            wuk32 = wuk_v.bitcast(jnp.uint32)
            rowj = row16 & 7
            lpar = lane16 & 1
            qa_slabs = []
            for g in range(4):
                z = None
                for ii in range(4):
                    i = 4 * g + ii
                    w = pltpu.bitcast(wuk32[pl.ds(i, DC, stride=16), :], BF16)
                    o = lax.dot_general(qs[g], w, (((1,), (1,)), ((), ())), preferred_element_type=F32)
                    o = jnp.where(rowj == 2 * ii + lpar, o, 0.0)
                    z = o if z is None else z + o
                zb = (z * (D ** -0.5)).astype(BF16)
                qa = jnp.concatenate(
                    [jnp.dot(zb[:, 256 * t:256 * (t + 1)], F0, preferred_element_type=F32) for t in range(4)], axis=1)
                qa_slabs.append(qa)
            qa_b = [jnp.concatenate([qa_slabs[g][8 * b:8 * b + 8] for g in range(4)], axis=0).astype(BF16) for b in range(B)]

        ctxc = []
        for b in range(B):
            qa = qa_b[b]

            def chunk_body(ci, carry, b=b, qa=qa):
                idx = b * NCH + ci
                cp_c(idx).wait()
                for t in range(NB):
                    m, l, acc = carry
                    start = pl.multiple_of(idx * CH + t * TB, TB)
                    c = ckv_v[pl.ds(start, TB), :]
                    s = lax.dot_general(qa, c, (((1,), (1,)), ((), ())), preferred_element_type=F32)
                    m_new = jnp.maximum(m, jnp.max(s, axis=1, keepdims=True))
                    alpha = jnp.exp(m - m_new)
                    p = jnp.exp(s - m_new)
                    l = alpha * l + jnp.sum(p, axis=1, keepdims=True)
                    acc = alpha * acc + jnp.dot(p.astype(BF16), c, preferred_element_type=F32)
                    carry = (m_new, l, acc)
                return carry

            init = (jnp.full((H, 1), -jnp.inf, F32), jnp.zeros((H, 1), F32), jnp.zeros((H, DC), F32))
            with scope("attn%d" % b):
                m, l, acc = lax.fori_loop(0, NCH, chunk_body, init)
            ctxc.append(acc / l)

        with scope("wait_wuv"):
            cp_wuv.wait()
        with scope("ctx"):
            wuv32 = wuv_v.bitcast(jnp.uint32)
            ctx_slabs = []
            for g in range(4):
                cg = jnp.concatenate([ctxc[b][8 * g:8 * g + 8] for b in range(B)], axis=0).astype(BF16)
                ce = jnp.where(par_mask, expand2(cg), 0.0).astype(BF16)
                acc = None
                for ii in range(4):
                    i = 4 * g + ii
                    w = pltpu.bitcast(wuv32[pl.ds(i, DC, stride=16), :], BF16)
                    o = jnp.dot(ce, w, preferred_element_type=F32)
                    o = jnp.where((row128 >> 1) == ii, o, 0.0)
                    acc = o if acc is None else acc + o
                ctx_slabs.append(acc)

        with scope("wait_w1"):
            cp_b1.wait()
            cp_b2.wait()
            cp_w1.wait()
        with scope("ffn1"):
            h = jnp.dot(xn16_bf, w1_v[...], preferred_element_type=F32) + b1_v[...].astype(F32)[None, :]
            h = jax.nn.gelu(h, approximate=True).astype(BF16)
        with scope("wait_w2"):
            cp_w2.wait()
        with scope("ffn2"):
            f = jnp.dot(h, w2_v[...], preferred_element_type=F32) + b2_v[...].astype(F32)[None, :]
            gate = f * jax.nn.sigmoid(f)

        s16 = jnp.zeros((16, M), F32)
        for ci in range(WO_CHUNKS):
            with scope("wait_wo%d" % ci):
                cp_o(ci).wait()
            with scope("wo%d" % ci):
                lhs = []
                for hh in range(HPC):
                    hd = ci * HPC + hh
                    lhs.append(jnp.where(row128 == (hd % 8), ctx_slabs[hd // 8], 0.0).astype(BF16))
                lhs = jnp.concatenate(lhs, axis=1)
                s16 = s16 + jnp.dot(lhs, wo_v[pl.ds(ci * HPC * D, HPC * D), :], preferred_element_type=F32)
        with scope("fin"):
            s0 = jnp.sum(s16[0:8], axis=0, keepdims=True)
            s1 = jnp.sum(s16[8:16], axis=0, keepdims=True)
            s = jnp.concatenate([s0, s1], axis=0)
            g2 = jnp.concatenate([gate[0:1], gate[8:9]], axis=0)
            o_ref[...] = (x + s * g2).astype(o_ref.dtype)

    return kernel, NCH


def make_fn(CH=2048, TB=512, WO_CHUNKS=8, scopes=False):
    kernel, NCH = make_kernel(CH, TB, WO_CHUNKS, scopes)

    def fn(A_x, A_c_kv, A_w_q, A_w_uk, A_w_uv, A_w_o, B_x, B_w1, B_b1, B_w2, B_b2):
        hbm = pl.BlockSpec(memory_space=pl.ANY)
        out = pl.pallas_call(
            kernel,
            out_shape=jax.ShapeDtypeStruct((B, M), A_x.dtype),
            in_specs=[hbm] * 10,
            out_specs=pl.BlockSpec(memory_space=pltpu.VMEM),
            scratch_shapes=[
                pltpu.VMEM((B, M), BF16),
                pltpu.VMEM((F,), BF16),
                pltpu.VMEM((M,), BF16),
                pltpu.VMEM((M * H, D), BF16),
                pltpu.VMEM((DC * H, D), BF16),
                pltpu.VMEM((B * SK, DC), BF16),
                pltpu.VMEM((DC * H, D), BF16),
                pltpu.VMEM((M, F), BF16),
                pltpu.VMEM((F, M), BF16),
                pltpu.VMEM((H * D, M), BF16),
                pltpu.SemaphoreType.DMA((8 + B * NCH + WO_CHUNKS,)),
            ],
            compiler_params=pltpu.CompilerParams(vmem_limit_bytes=100 * 1024 * 1024),
        )(A_x.reshape(B, M), A_c_kv.reshape(B * SK, DC), A_w_q.reshape(M * H, D), A_w_uk.reshape(DC * H, D),
          A_w_uv.reshape(DC * H, D), A_w_o.reshape(H * D, M), B_w1, B_b1, B_w2, B_b2)
        return out.reshape(B, 1, M)
    return fn


@jax.jit
def pallas_recurrent_scan__compressed_kv_cla__dense_activation_gelu__decode_kernel(
    A_x: jax.Array,
    A_c_kv: jax.Array,
    A_w_q: jax.Array,
    A_w_uk: jax.Array,
    A_w_uv: jax.Array,
    A_w_o: jax.Array,
    B_x: jax.Array,
    B_w1: jax.Array,
    B_b1: jax.Array,
    B_w2: jax.Array,
    B_b2: jax.Array,
):
    return make_fn()(A_x, A_c_kv, A_w_q, A_w_uk, A_w_uv, A_w_o, B_x, B_w1, B_b1, B_w2, B_b2)
```

```python
import jax
import jax.numpy as jnp
from jax import lax
import jax.experimental.pallas as pl
import jax.experimental.pallas.tpu as pltpu

F32, BF16 = jnp.float32, jnp.bfloat16

B, H, D, M, SK, DC, F = 2, 32, 128, 512, 16384, 512, 1792
TB = 1024
KV_CHUNKS = (16384, 10240, 6144)
WO_CHUNKS = (16, 8, 4, 2, 1, 1)
WO_STEP = 2
WO_PEELED = 2
NSEM = 3

NBLK = SK // TB
KV_START = [sum(KV_CHUNKS[:i]) for i in range(len(KV_CHUNKS))]
WO_START = [sum(WO_CHUNKS[:i]) for i in range(len(WO_CHUNKS))]
WO_LOOP_HEADS = sum(WO_CHUNKS[:len(WO_CHUNKS) - WO_PEELED])
assert sum(KV_CHUNKS) == B * SK and all(s % TB == 0 for s in KV_START)
assert sum(WO_CHUNKS) == H and all(s % WO_STEP == 0 for s in WO_START if s <= WO_LOOP_HEADS)


def _kernel(x_hbm, ckv_hbm, wq_hbm, wuk_hbm, wuv_hbm, wo_hbm, w1_hbm, b1_hbm, w2_hbm, b2_hbm,
            o_ref,
            x_v, b1_v, b2_v, wq_v, wuk_v, ckv_v, wuv_v, w1_v, w2_v, wo_v,
            q_s, z_s, qa_s, cc_s, ce_s, ctx_s, lhs_s, s_s, sems):
    def rows(hbm, vmem, lo, n):
        return hbm.at[pl.ds(lo, n)], vmem.at[pl.ds(lo, n)]

    groups = [[(x_hbm, x_v), (b1_hbm, b1_v), (b2_hbm, b2_v)], [(wq_hbm, wq_v)], [(wuk_hbm, wuk_v)]]
    groups += [[rows(ckv_hbm, ckv_v, lo, n)] for lo, n in zip(KV_START, KV_CHUNKS)]
    groups += [[(wuv_hbm, wuv_v)], [(w1_hbm, w1_v), (w2_hbm, w2_v)]]
    groups += [[rows(wo_hbm, wo_v, lo * D, n * D)] for lo, n in zip(WO_START, WO_CHUNKS)]
    G_X, G_WQ, G_WUK, G_KV = 0, 1, 2, 3
    G_WUV = G_KV + len(KV_CHUNKS)
    G_FFN, G_WO = G_WUV + 1, G_WUV + 2

    def start(k):
        if k < len(groups):
            for src, dst in groups[k]:
                pltpu.make_async_copy(src, dst, sems.at[k % NSEM]).start()

    def wait(k):
        for src, dst in groups[k]:
            pltpu.make_async_copy(src, dst, sems.at[k % NSEM]).wait()
        start(k + NSEM)

    for k in range(NSEM):
        start(k)

    def iota(shape, dim):
        return lax.broadcasted_iota(jnp.int32, shape, dim)

    dup = jnp.where((iota((128, 256), 1) >> 1) == iota((128, 256), 0), 1.0, 0.0).astype(BF16)
    fold = jnp.where((iota((256, 128), 0) >> 1) == iota((256, 128), 1), 1.0, 0.0).astype(BF16)
    row_j = iota((16, 1024), 0) & 7
    lane_par = iota((16, 1024), 1) & 1
    row_pair = iota((16, D), 0) >> 1 & 3

    def dot(a, b):
        return jnp.dot(a, b, preferred_element_type=F32)

    def dot_t(a, b):
        return lax.dot_general(a, b, (((1,), (1,)), ((), ())), preferred_element_type=F32)

    def pair_rows(w32, g, ii):
        sub = w32.at[pl.ds(pl.multiple_of(4 * g, 4), 16 * 511 + 4)]
        return pltpu.bitcast(sub[pl.ds(ii, 512, stride=16), :], BF16)

    def by_parity(a):
        wide = jnp.concatenate([dot(a[:, 128 * t:128 * (t + 1)], dup) for t in range(4)], axis=1)
        return jnp.where((row_j & 1) == lane_par, wide, 0.0).astype(BF16)

    def per_head(lhs_of, w32, out_s):
        def body(g, _):
            lhs = lhs_of(g)
            acc = dot(lhs, pair_rows(w32, g, 0))
            for ii in range(1, 4):
                acc = jnp.where(row_pair == ii, dot(lhs, pair_rows(w32, g, ii)), acc)
            out_s[g] = acc
            return 0
        lax.fori_loop(0, 4, body, 0)

    wait(G_X)
    x = x_v[...].astype(F32)
    xc = x - jnp.mean(x, axis=-1, keepdims=True)
    xn = xc / jnp.sqrt(jnp.mean(xc * xc, axis=-1, keepdims=True) + 1e-5)
    xn16 = by_parity(jnp.concatenate([jnp.broadcast_to(xn[b:b + 1], (8, M)) for b in range(B)], axis=0).astype(BF16))
    xn8 = jnp.concatenate([xn, jnp.zeros((8 - B, M), F32)], axis=0).astype(BF16)

    wait(G_WQ)
    per_head(lambda g: xn16, wq_v.bitcast(jnp.uint32), q_s)

    wait(G_WUK)
    wuk32 = wuk_v.bitcast(jnp.uint32)

    def qlat_body(g, _):
        qg = q_s[g].astype(BF16)
        z = jnp.zeros((16, 1024), F32)
        for ii in range(4):
            z = jnp.where(row_j == 2 * ii + lane_par, dot_t(qg, pair_rows(wuk32, g, ii)), z)
        z_s[g] = z
        return 0
    lax.fori_loop(0, 4, qlat_body, 0)
    zb = (z_s[...].reshape(64, 1024) * (D ** -0.5)).astype(BF16)
    qa = jnp.concatenate([dot(zb[:, 256 * t:256 * (t + 1)], fold) for t in range(4)], axis=1)
    for b in range(B):
        qa_s[b] = jnp.concatenate([qa[16 * g + 8 * b:16 * g + 8 * b + 8] for g in range(4)], axis=0).astype(BF16)

    def kv_block(j):
        return ckv_v[pl.ds(pl.multiple_of(j * TB, TB), TB), :]

    def batch_body(b, _):
        q_lat = qa_s[b]

        def body(j, carry):
            m, l, acc, p_prev, a_prev = carry
            gj = b * NBLK + j
            for i, lo in enumerate(KV_START):
                @pl.when(gj == lo // TB)
                def _():
                    wait(G_KV + i)
            s = dot_t(q_lat, kv_block(gj))
            acc = a_prev * acc + dot(p_prev, kv_block(jnp.maximum(gj - 1, b * NBLK)))
            m_new = jnp.maximum(m, jnp.max(s, axis=1, keepdims=True))
            alpha = jnp.exp(m - m_new)
            p = jnp.exp(s - m_new)
            l = alpha * l + jnp.sum(p, axis=1, keepdims=True)
            return m_new, l, acc, p.astype(BF16), alpha

        init = (jnp.full((H, 1), -jnp.inf, F32), jnp.zeros((H, 1), F32), jnp.zeros((H, DC), F32),
                jnp.zeros((H, TB), BF16), jnp.zeros((H, 1), F32))
        _, l, acc, p_prev, a_prev = lax.fori_loop(0, NBLK, body, init)
        acc = a_prev * acc + dot(p_prev, kv_block((b + 1) * NBLK - 1))
        cc_s[b] = acc / l
        return 0
    lax.fori_loop(0, B, batch_body, 0)

    for g in range(4):
        ce_s[g] = by_parity(jnp.concatenate([cc_s[b, 8 * g:8 * g + 8] for b in range(B)], axis=0).astype(BF16))
    wait(G_WUV)
    per_head(lambda g: ce_s[g], wuv_v.bitcast(jnp.uint32), ctx_s)
    ctx = ctx_s[...].reshape(64, D)
    r8 = iota((8, D), 0)
    for h in range(H):
        r = 16 * (h // 8) + h % 8
        v = jnp.where(r8 == 0, jnp.broadcast_to(ctx[r:r + 1], (8, D)),
                      jnp.where(r8 == 1, jnp.broadcast_to(ctx[r + 8:r + 9], (8, D)), 0.0))
        lhs_s[h // WO_STEP, :, (h % WO_STEP) * D:(h % WO_STEP + 1) * D] = v.astype(BF16)

    wait(G_FFN)
    hid = jax.nn.gelu(dot(xn8, w1_v[...]) + b1_v[...].astype(F32)[None, :], approximate=True).astype(BF16)
    f = dot(hid, w2_v[...]) + b2_v[...].astype(F32)[None, :]
    gate = (f * jax.nn.sigmoid(f))[0:B]

    s_s[...] = jnp.zeros((8, M), F32)

    def wo_body(i, _):
        for k in range(len(WO_CHUNKS) - WO_PEELED):
            @pl.when(i == WO_START[k] // WO_STEP)
            def _():
                wait(G_WO + k)
        w = wo_v[pl.ds(pl.multiple_of(i * (WO_STEP * D), WO_STEP * D), WO_STEP * D), :]
        s_s[...] += dot(lhs_s[i], w)
        return 0
    lax.fori_loop(0, WO_LOOP_HEADS // WO_STEP, wo_body, 0)
    for k in range(len(WO_CHUNKS) - WO_PEELED, len(WO_CHUNKS)):
        h0, n = WO_START[k], WO_CHUNKS[k]
        wait(G_WO + k)
        lhs = lhs_s[h0 // WO_STEP, :, (h0 % WO_STEP) * D:(h0 % WO_STEP + n) * D]
        s_s[...] += dot(lhs, wo_v[h0 * D:(h0 + n) * D, :])
    o_ref[...] = (x + s_s[0:B] * gate).astype(o_ref.dtype)


@jax.jit
def pallas_recurrent_scan__compressed_kv_cla__dense_activation_gelu__decode_kernel(
    A_x: jax.Array,
    A_c_kv: jax.Array,
    A_w_q: jax.Array,
    A_w_uk: jax.Array,
    A_w_uv: jax.Array,
    A_w_o: jax.Array,
    B_x: jax.Array,
    B_w1: jax.Array,
    B_b1: jax.Array,
    B_w2: jax.Array,
    B_b2: jax.Array,
):
    del B_x
    hbm = pl.BlockSpec(memory_space=pl.ANY)
    out = pl.pallas_call(
        _kernel,
        out_shape=jax.ShapeDtypeStruct((B, M), A_x.dtype),
        in_specs=[hbm] * 10,
        out_specs=pl.BlockSpec(memory_space=pltpu.VMEM),
        scratch_shapes=[
            pltpu.VMEM((B, M), BF16),
            pltpu.VMEM((F,), BF16),
            pltpu.VMEM((M,), BF16),
            pltpu.VMEM((M * H, D), BF16),
            pltpu.VMEM((DC * H, D), BF16),
            pltpu.VMEM((B * SK, DC), BF16),
            pltpu.VMEM((DC * H, D), BF16),
            pltpu.VMEM((M, F), BF16),
            pltpu.VMEM((F, M), BF16),
            pltpu.VMEM((H * D, M), BF16),
            pltpu.VMEM((4, 16, D), F32),
            pltpu.VMEM((4, 16, 1024), F32),
            pltpu.VMEM((B, H, DC), BF16),
            pltpu.VMEM((B, H, DC), F32),
            pltpu.VMEM((4, 16, 1024), BF16),
            pltpu.VMEM((4, 16, D), F32),
            pltpu.VMEM((H // WO_STEP, 8, WO_STEP * D), BF16),
            pltpu.VMEM((8, M), F32),
            pltpu.SemaphoreType.DMA((NSEM,)),
        ],
        compiler_params=pltpu.CompilerParams(vmem_limit_bytes=100 * 1024 * 1024),
    )(A_x.reshape(B, M), A_c_kv.reshape(B * SK, DC), A_w_q.reshape(M * H, D), A_w_uk.reshape(DC * H, D),
      A_w_uv.reshape(DC * H, D), A_w_o.reshape(H * D, M), B_w1, B_b1, B_w2, B_b2)
    return out.reshape(B, 1, M)
```
